```python
import jax
import jax.numpy as jnp

def _softmax(x, axis=-1):
    return jax.nn.softmax(x, axis=axis)

def _gelu(x):
    return jax.nn.gelu(x, approximate=True)

def _silu(x):
    return jax.nn.silu(x)

def _sigmoid(x):
    return jax.nn.sigmoid(x)

def _layernorm(x, axis=-1, eps=1e-05):
    m = jnp.mean(x, axis=axis, keepdims=True)
    v = jnp.var(x, axis=axis, keepdims=True)
    return (x - m) / jnp.sqrt(v + eps)

def _scatter_add(tgt, idx, src, axis=0):
    return tgt.at[idx].add(src)

def _segment_sum(src, seg, n):
    return jax.ops.segment_sum(src, seg, n)

class _Rng:

    def __init__(self, key):
        self._k = key

    def _next(self):
        self._k, sub = jax.random.split(self._k)
        return sub

    def normal(self, shape):
        return jax.random.normal(self._next(), shape, dtype=jnp.bfloat16)

    def randint(self, lo, hi, shape):
        return jax.random.randint(self._next(), shape, lo, hi, dtype=jnp.int32)

    def uniform(self, shape, lo=0.0, hi=1.0):
        return jax.random.uniform(self._next(), shape, jnp.bfloat16, lo, hi)

    def permutation(self, n):
        return jax.random.permutation(self._next(), n)
kernel_name = 'gated_mix__memory_aug_recurrent_mem_tr__ssm_conv_h3__prompt'

def setup_inputs():
    _rng = _Rng(jax.random.key(int.from_bytes(__import__("os").urandom(4), "little")))
    _w = lambda a: (lambda t: t.astype(jnp.bfloat16) if jnp.issubdtype(t.dtype, jnp.floating) else t)(jnp.asarray(a))

    def _A_setup():
        B, S, Dm = (1, 2048, 640)
        H, Dh = (32, 192)
        M, seg = (8, 32)
        seg = min(seg, S)
        S = S // seg * seg
        return {'x': _w((lambda *s: _rng.normal(s) * 0.05)(B, S, Dm)), 'mem0': _w((lambda *s: _rng.normal(s) * 0.05)(B, M, Dm)), 'Wq': _w((lambda *s: _rng.normal(s) * 0.05)(Dm, H, Dh) * Dm ** (-0.5)), 'Wk': _w((lambda *s: _rng.normal(s) * 0.05)(Dm, H, Dh) * Dm ** (-0.5)), 'Wv': _w((lambda *s: _rng.normal(s) * 0.05)(Dm, H, Dh) * Dm ** (-0.5)), 'Wo': _w((lambda *s: _rng.normal(s) * 0.05)(H, Dh, Dm) * (H * Dh) ** (-0.5)), 'seg_len': seg}
    _A_in = _A_setup()

    def _B_setup():
        B, S, D = (1, 2048, 640)
        ks = 4
        return {'q': _w((lambda *s: _rng.normal(s) * 0.05)(B, S, D)), 'k': _w((lambda *s: _rng.normal(s) * 0.05)(B, S, D)), 'v': _w((lambda *s: _rng.normal(s) * 0.05)(B, S, D)), 'shift_k': _w((lambda *s: _rng.normal(s) * 0.05)(D, ks) * 0.5), 'ssm_k': _w((lambda *s: _rng.normal(s) * 0.05)(D, S) * (1.0 / S ** 0.5)), 'ssm_D': _w((lambda *s: _rng.normal(s) * 0.05)(D))}
    _B_in = _B_setup()
    return {'A_x': _A_in['x'], 'A_mem0': _A_in['mem0'], 'A_Wq': _A_in['Wq'], 'A_Wk': _A_in['Wk'], 'A_Wv': _A_in['Wv'], 'A_Wo': _A_in['Wo'], 'A_seg_len': _A_in['seg_len'], 'B_q': _B_in['q'], 'B_k': _B_in['k'], 'B_v': _B_in['v'], 'B_shift_k': _B_in['shift_k'], 'B_ssm_k': _B_in['ssm_k'], 'B_ssm_D': _B_in['ssm_D'], 'gate_w': _w((lambda *s: _rng.normal(s) * 0.05)(640))}

def reference(A_x, A_mem0, A_Wq, A_Wk, A_Wv, A_Wo, A_seg_len, B_q, B_k, B_v, B_shift_k, B_ssm_k, B_ssm_D, gate_w):

    def _A_ref(x, mem0, Wq, Wk, Wv, Wo, seg_len):
        B, S, Dm = x.shape
        H, Dh = (Wq.shape[1], Wq.shape[2])
        M = mem0.shape[1]
        scale = Dh ** (-0.5)
        n_seg = S // seg_len
        L = M + seg_len
        idx = jnp.arange(L)
        mask = (idx[:, None] < M) | (idx[:, None] >= idx[None, :])
        mem = mem0
        outs = []
        for s in range(n_seg):
            xs = x[:, s * seg_len:(s + 1) * seg_len, :].copy()
            h = jnp.concatenate([mem, xs], axis=1)
            q = jnp.einsum('btd,dhe->bhte', h, Wq)
            k = jnp.einsum('btd,dhe->bhte', h, Wk)
            v = jnp.einsum('btd,dhe->bhte', h, Wv)
            scores = jnp.einsum('bhqe,bhke->bhqk', q, k) * scale
            scores = jnp.where(mask[None, None], scores, -1000000000.0)
            p = _softmax(scores, axis=-1)
            o = jnp.einsum('bhqk,bhke->bhqe', p, v)
            o = jnp.einsum('bhte,hed->btd', o, Wo)
            mem = o[:, :M, :].copy()
            outs.append(o[:, M:, :])
        return jnp.concatenate(outs, axis=1)

    def _B_ref(q, k, v, shift_k, ssm_k, ssm_D):
        B, S, D = q.shape
        ks = shift_k.shape[-1]
        k_pad = jnp.pad(k, ((0, 0), (ks - 1, 0), (0, 0)))
        k_shift = jnp.zeros_like(k)
        for t in range(ks):
            k_shift = k_shift + k_pad[:, t:t + S, :] * shift_k[:, ks - 1 - t][None, None, :]
        kv = k_shift * v
        L = 2 * S
        kv_pad = jnp.pad(kv, ((0, 0), (0, S), (0, 0)))
        kf_pad = jnp.pad(ssm_k, ((0, 0), (0, S)))
        kv_f = (lambda x, axes=(-2, -1): jnp.fft.rfft2(x.astype(jnp.float32), axes=axes))(kv_pad[:, None, :, :], axes=(1, 2))
        kf_f = (lambda x, axes=(-2, -1): jnp.fft.rfft2(x.astype(jnp.float32), axes=axes))(kf_pad[:, None, :], axes=(1, 2))
        kf_f = (lambda x, *d: x.transpose(*d))(kf_f, 1, 2, 0)
        y_f = kv_f * kf_f[None, :, :, :]
        y = (lambda x, s, axes=(-2, -1): jnp.fft.irfft2(x, s=s, axes=axes).astype(jnp.bfloat16))(y_f, (1, L), axes=(1, 2))[:, 0, :S, :]
        y = y + kv * ssm_D[None, None, :]
        return q * y
    x = A_x
    g = _sigmoid((x * gate_w).sum(-1, keepdims=True))
    a = _A_ref(x, A_mem0, A_Wq, A_Wk, A_Wv, A_Wo, A_seg_len)
    b = _B_ref(x, B_k, B_v, B_shift_k, B_ssm_k, B_ssm_D)
    return g * a + (1 - g) * b
```

```python
import functools

import jax
import jax.numpy as jnp
import numpy as np
from jax import lax
from jax.experimental import pallas as pl
from jax.experimental.pallas import tpu as pltpu

F32 = jnp.float32
BF16 = jnp.bfloat16
LANES = 128
CHUNK = 128

_NN = (((1,), (0,)), ((), ()))
_NT = (((1,), (1,)), ((), ()))


def _dot(a, b, dims=_NN):
    return lax.dot_general(a, b, dims, preferred_element_type=F32)


def _dft_matrices():
    k = np.arange(CHUNK, dtype=np.float64)[:, None]
    n = np.arange(CHUNK, dtype=np.float64)[None, :]
    theta = np.pi * (2.0 * k + 1.0) * n / (2.0 * CHUNK)
    fwd = np.concatenate([np.cos(theta), -np.sin(theta)], axis=0)
    inv = fwd.T / CHUNK
    return np.asarray(fwd, dtype=BF16), np.asarray(inv, dtype=BF16)


def _kernel(
    x_hbm, k_hbm, v_hbm, h_hbm, wq_hbm, wk_hbm, wv_hbm, wo_hbm,
    mem0_ref, shift_ref, dvec_ref, gw_ref, fwd_ref, inv_ref,
    out_hbm,
    xs, ks, vs, hs, wraw, wqkv, wo, kpad, kvf, kvb, uspec, gspec, pspec, bterm, obuf,
    in_sems, w_sems, out_sem,
    *, seg, n_mem, n_taps, head_dim,
):
    n_ct, seq, _ = xs.shape
    n_pairs = wo.shape[0]
    pw = 2 * head_dim
    n_seg = seq // seg
    n_chunks = seq // CHUNK
    rows = n_mem + seg
    scale = head_dim ** (-0.5)

    def in_copy(which, c):
        cols = pl.ds(c * LANES, LANES)
        src = (k_hbm.at[:, cols], v_hbm.at[:, cols], h_hbm.at[cols, :], x_hbm.at[:, cols])[which]
        dst = (ks, vs, hs, xs)[which].at[c]
        return pltpu.make_async_copy(src, dst, in_sems.at[which, c])

    def w_copy(which, p):
        src = (wq_hbm, wk_hbm, wv_hbm, wo_hbm)[which]
        return pltpu.make_async_copy(
            src.at[pl.ds(p * pw, pw), :], wraw.at[which, p], w_sems.at[which, p])

    for c in range(n_ct):
        for which in range(4):
            in_copy(which, c).start()
    for p in range(n_pairs):
        for which in range(4):
            w_copy(which, p).start()

    kpad[pl.ds(0, 8), :] = jnp.zeros((8, LANES), F32)
    sub = lax.broadcasted_iota(jnp.int32, (8, LANES), 0)
    sgn = jnp.where((sub & 1) == 0, 1.0, -1.0).astype(F32)

    def b_tile(c, carry):
        cols = pl.ds(pl.multiple_of(c * LANES, LANES), LANES)
        pltpu.make_async_copy(ks.at[c], ks.at[c], in_sems.at[0, c]).wait()
        pltpu.make_async_copy(vs.at[c], vs.at[c], in_sems.at[1, c]).wait()
        kpad[pl.ds(8, seq), :] = ks[c].astype(F32)
        taps = shift_ref[:, cols].astype(F32)
        for a in range(n_chunks):
            acc = kpad[pl.ds(8 + a * CHUNK, CHUNK), :] * taps[0:1, :]
            for j in range(1, n_taps):
                acc = acc + kpad[pl.ds(8 + a * CHUNK - j, CHUNK), :] * taps[j:j + 1, :]
            kv = acc * vs[c, pl.ds(a * CHUNK, CHUNK), :].astype(F32)
            kvf[pl.ds(a * CHUNK, CHUNK), :] = kv
            kvb[:, pl.ds(a * CHUNK, CHUNK)] = kv.astype(BF16)
        uspec[...] = _dot(fwd_ref[...], kvb[...])

        pltpu.make_async_copy(hs.at[c], hs.at[c], in_sems.at[2, c]).wait()
        hcat = jnp.concatenate(
            [hs[c, :, pl.ds(a * CHUNK, CHUNK)] for a in range(n_chunks)], axis=0)
        gspec[...] = _dot(fwd_ref[...], hcat, _NT)

        def freq_group(r, carry2):
            re = pl.ds(pl.multiple_of(r * 8, 8), 8)
            im = pl.ds(pl.multiple_of(CHUNK + r * 8, 8), 8)
            col = lambda a: pl.ds(a * LANES, LANES)
            g_re, g_im = [], []
            for a in range(n_chunks):
                gr, gi = gspec[re, col(a)], gspec[im, col(a)]
                if a > 0:
                    gr = gr - sgn * gspec[im, col(a - 1)]
                    gi = gi + sgn * gspec[re, col(a - 1)]
                g_re.append(gr)
                g_im.append(gi)
            for a in range(n_chunks):
                pr = pi = None
                for b in range(a + 1):
                    ur, ui = uspec[re, col(b)], uspec[im, col(b)]
                    tr = ur * g_re[a - b] - ui * g_im[a - b]
                    ti = ur * g_im[a - b] + ui * g_re[a - b]
                    pr = tr if pr is None else pr + tr
                    pi = ti if pi is None else pi + ti
                pspec[re, col(a)] = pr
                pspec[im, col(a)] = pi
            return carry2

        lax.fori_loop(0, CHUNK // 8, freq_group, 0)

        y = _dot(inv_ref[...], pspec[...].astype(BF16))
        pltpu.make_async_copy(xs.at[c], xs.at[c], in_sems.at[3, c]).wait()
        dvec = dvec_ref[:, cols].astype(F32)
        for a in range(n_chunks):
            t = pl.ds(a * CHUNK, CHUNK)
            ya = y[:, a * LANES:(a + 1) * LANES] + kvf[t, :] * dvec
            bterm[c, t, :] = xs[c, t, :].astype(F32) * ya
        return carry

    lax.fori_loop(0, n_ct, b_tile, 0)

    def w_pair(p, carry):
        for which in range(3):
            pltpu.make_async_copy(
                wraw.at[which, p], wraw.at[which, p], w_sems.at[which, p]).wait()
            wqkv[p, which] = pltpu.bitcast(wraw[which, p].T, jnp.uint32)
        pltpu.make_async_copy(wraw.at[3, p], wraw.at[3, p], w_sems.at[3, p]).wait()
        wo[p] = pltpu.bitcast(wraw[3, p], jnp.uint32)
        return carry

    lax.fori_loop(0, n_pairs, w_pair, 0)

    lane = lax.broadcasted_iota(jnp.int32, (rows, LANES), 1)
    lane_lo = lane < (head_dim - LANES)
    col = lax.broadcasted_iota(jnp.int32, (rows, 2 * rows), 1)
    row = lax.broadcasted_iota(jnp.int32, (rows, 2 * rows), 0)
    first = col < rows
    key = jnp.where(first, col, col - rows)
    visible = (row < n_mem) | (row >= key)
    zeros = jnp.zeros((rows, LANES), F32)
    gate_w = gw_ref[...].astype(F32)

    def split_heads(t):
        a, b, c = t[:, :LANES], t[:, LANES:2 * LANES], t[:, 2 * LANES:]
        top = jnp.concatenate([a, jnp.where(lane_lo, b, 0.0), zeros], axis=1)
        bot = jnp.concatenate([zeros, jnp.where(lane_lo, 0.0, b), c], axis=1)
        return jnp.concatenate([top, bot], axis=0).astype(BF16)

    def softmax_pair(s):
        s = jnp.where(visible, s * scale, -1000000000.0)
        m0 = jnp.max(jnp.where(first, s, -jnp.inf), axis=1, keepdims=True)
        m1 = jnp.max(jnp.where(first, -jnp.inf, s), axis=1, keepdims=True)
        e = jnp.exp(s - jnp.where(first, m0, m1))
        l0 = jnp.sum(jnp.where(first, e, 0.0), axis=1, keepdims=True)
        l1 = jnp.sum(jnp.where(first, 0.0, e), axis=1, keepdims=True)
        return e / jnp.where(first, l0, l1)

    def step(s, mem):
        t = pl.ds(pl.multiple_of(s * seg, seg), seg)
        xt = jnp.concatenate([xs[c, t, :].astype(F32) for c in range(n_ct)], axis=1)
        h = jnp.concatenate([mem, xt], axis=0)

        def proj(p, which):
            return _dot(h, pltpu.bitcast(wqkv[p, which], BF16))

        q, k, v, prob, o = {}, {}, {}, {}, {}
        acc = None
        for i in range(n_pairs + 2):
            if i < n_pairs:
                q[i] = proj(i, 0)
            if 0 <= i - 1 < n_pairs:
                prob[i - 1] = softmax_pair(_dot(q.pop(i - 1), k.pop(i - 1), _NT))
            if i < n_pairs:
                k[i] = split_heads(proj(i, 1))
                v[i] = split_heads(proj(i, 2))
            if 0 <= i - 1 < n_pairs:
                o[i - 1] = _dot(prob.pop(i - 1), v.pop(i - 1))
            if 0 <= i - 2 < n_pairs:
                part = _dot(o.pop(i - 2), pltpu.bitcast(wo[i - 2], BF16))
                acc = part if acc is None else acc + part

        gate = jax.nn.sigmoid(jnp.sum(xt * gate_w, axis=1, keepdims=True))
        b = jnp.concatenate([bterm[c, t, :] for c in range(n_ct)], axis=1)
        res = gate * acc[n_mem:, :] + (1.0 - gate) * b
        obuf[t, :] = res.astype(BF16)
        pltpu.make_async_copy(obuf.at[t, :], out_hbm.at[t, :], out_sem).start()
        return acc[:n_mem, :].astype(BF16).astype(F32)

    lax.fori_loop(0, n_seg, step, mem0_ref[...].astype(F32))
    pltpu.make_async_copy(obuf, out_hbm, out_sem).wait()


@functools.partial(jax.jit, static_argnames=("A_seg_len",))
def pallas_gated_mix__memory_aug_recurrent_mem_tr__ssm_conv_h3__prompt_kernel(
    A_x: jax.Array,
    A_mem0: jax.Array,
    A_Wq: jax.Array,
    A_Wk: jax.Array,
    A_Wv: jax.Array,
    A_Wo: jax.Array,
    A_seg_len: int,
    B_q: jax.Array,
    B_k: jax.Array,
    B_v: jax.Array,
    B_shift_k: jax.Array,
    B_ssm_k: jax.Array,
    B_ssm_D: jax.Array,
    gate_w: jax.Array,
):
    del B_q
    batch, seq, dm = A_x.shape
    _, n_heads, head_dim = A_Wq.shape
    n_mem = A_mem0.shape[1]
    n_taps = B_shift_k.shape[1]
    seg = int(A_seg_len)
    assert batch == 1 and head_dim == 192 and n_heads % 2 == 0 and dm % LANES == 0
    assert seq % seg == 0 and seq % CHUNK == 0 and seg % 16 == 0 and n_mem % 8 == 0
    assert 2 * (seg + n_mem) <= LANES and n_taps <= 8
    n_ct = dm // LANES
    n_pairs = n_heads // 2
    pw = 2 * head_dim
    n_chunks = seq // CHUNK

    as_rows = lambda w: jnp.transpose(w, (1, 2, 0)).reshape(n_heads * head_dim, dm)
    fwd, inv = _dft_matrices()

    hbm = pl.BlockSpec(memory_space=pl.ANY)
    vmem = pl.BlockSpec(memory_space=pltpu.VMEM)
    out = pl.pallas_call(
        functools.partial(_kernel, seg=seg, n_mem=n_mem, n_taps=n_taps, head_dim=head_dim),
        out_shape=jax.ShapeDtypeStruct((seq, dm), BF16),
        in_specs=[hbm] * 8 + [vmem] * 6,
        out_specs=hbm,
        scratch_shapes=[
            pltpu.VMEM((n_ct, seq, LANES), BF16),
            pltpu.VMEM((n_ct, seq, LANES), BF16),
            pltpu.VMEM((n_ct, seq, LANES), BF16),
            pltpu.VMEM((n_ct, LANES, seq), BF16),
            pltpu.VMEM((4, n_pairs, pw, dm), BF16),
            pltpu.VMEM((n_pairs, 3, dm // 2, pw), jnp.uint32),
            pltpu.VMEM((n_pairs, pw // 2, dm), jnp.uint32),
            pltpu.VMEM((seq + 8, LANES), F32),
            pltpu.VMEM((seq, LANES), F32),
            pltpu.VMEM((CHUNK, n_chunks * LANES), BF16),
            pltpu.VMEM((2 * CHUNK, n_chunks * LANES), F32),
            pltpu.VMEM((2 * CHUNK, n_chunks * LANES), F32),
            pltpu.VMEM((2 * CHUNK, n_chunks * LANES), F32),
            pltpu.VMEM((n_ct, seq, LANES), F32),
            pltpu.VMEM((seq, dm), BF16),
            pltpu.SemaphoreType.DMA((4, n_ct)),
            pltpu.SemaphoreType.DMA((4, n_pairs)),
            pltpu.SemaphoreType.DMA,
        ],
        compiler_params=pltpu.CompilerParams(vmem_limit_bytes=110 * 1024 * 1024),
        name="gated_mix_rmt_h3",
    )(
        A_x.reshape(seq, dm), B_k.reshape(seq, dm), B_v.reshape(seq, dm), B_ssm_k,
        as_rows(A_Wq), as_rows(A_Wk), as_rows(A_Wv), A_Wo.reshape(n_heads * head_dim, dm),
        A_mem0.reshape(n_mem, dm), B_shift_k.T, B_ssm_D.reshape(1, dm), gate_w.reshape(1, dm),
        fwd, inv,
    )
    return out.reshape(batch, seq, dm)
```

```python
import functools

import jax
import jax.numpy as jnp
import numpy as np
from jax import lax
from jax.experimental import pallas as pl
from jax.experimental.pallas import tpu as pltpu

F32 = jnp.float32
BF16 = jnp.bfloat16
LANES = 128
CHUNK = 128

_NN = (((1,), (0,)), ((), ()))
_NT = (((1,), (1,)), ((), ()))


def _dot(a, b, dims=_NN):
    return lax.dot_general(a, b, dims, preferred_element_type=F32)


def _dft_matrices():
    k = np.arange(CHUNK, dtype=np.float64)[:, None]
    n = np.arange(CHUNK, dtype=np.float64)[None, :]
    theta = np.pi * (2.0 * k + 1.0) * n / (2.0 * CHUNK)
    fwd = np.concatenate([np.cos(theta), -np.sin(theta)], axis=0)
    inv = fwd.T / CHUNK
    return np.asarray(fwd, dtype=BF16), np.asarray(inv, dtype=BF16)


def _mxu_order(n, lag=6):
    order = []
    for i in range(n):
        order += [("q", i), ("pv", i - 2), ("s", i - 1), ("k", i), ("v", i), ("o", i - lag)]
    held = [("o", i) for i in range(n - lag, n)]
    order += held[:1] + [("pv", n - 2), ("s", n - 1)] + held[1:-2] + [("pv", n - 1)] + held[-2:]
    return [(op, i) for op, i in order if i >= 0]


def _kernel(
    x_hbm, k_hbm, v_hbm, h_hbm, wq_hbm, wk_hbm, wv_hbm, wo_hbm,
    mem0_ref, shift_ref, dvec_ref, gw_ref, fwd_ref, inv_ref,
    out_hbm,
    xs, ks, vs, hs, wraw, wqkv, wo, kpad, kvf, kvb, uspec, gspec, pspec, bterm, obuf,
    in_sems, w_sems, out_sem,
    *, seg, n_mem, n_taps, head_dim,
):
    n_ct, seq, _ = xs.shape
    n_pairs = wo.shape[0]
    pw = 2 * head_dim
    n_seg = seq // seg
    n_chunks = seq // CHUNK
    rows = n_mem + seg
    scale = head_dim ** (-0.5)

    def in_copy(which, c):
        cols = pl.ds(pl.multiple_of(c * LANES, LANES), LANES)
        src = (k_hbm.at[:, cols], v_hbm.at[:, cols], h_hbm.at[cols, :], x_hbm.at[:, cols])[which]
        dst = (ks, vs, hs, xs)[which].at[c]
        return pltpu.make_async_copy(src, dst, in_sems.at[which, c])

    def w_copy(which, p):
        src = (wq_hbm, wk_hbm, wv_hbm, wo_hbm)[which]
        return pltpu.make_async_copy(
            src.at[pl.ds(pl.multiple_of(p * pw, pw), pw), :], wraw.at[which, p], w_sems.at[which, p])

    def start_inputs(c):
        for which in range(4):
            in_copy(which, c).start()

    def start_weights(p):
        for which in range(4):
            w_copy(which, p).start()

    start_inputs(0)
    start_inputs(1)

    kpad[pl.ds(0, 8), :] = jnp.zeros((8, LANES), F32)
    sub = lax.broadcasted_iota(jnp.int32, (8, LANES), 0)
    sgn = jnp.where((sub & 1) == 0, 1.0, -1.0).astype(F32)

    def b_tile(c, carry):
        cols = pl.ds(pl.multiple_of(c * LANES, LANES), LANES)
        pltpu.make_async_copy(ks.at[c], ks.at[c], in_sems.at[0, c]).wait()
        pltpu.make_async_copy(vs.at[c], vs.at[c], in_sems.at[1, c]).wait()

        @pl.when(c + 2 < n_ct)
        def _():
            start_inputs(c + 2)
            start_weights(c)

        @pl.when(c + 2 >= n_ct)
        def _():
            start_weights(2 * c - (n_ct - 2))
            start_weights(2 * c - (n_ct - 2) + 1)

        kpad[pl.ds(8, seq), :] = ks[c].astype(F32)
        taps = shift_ref[:, cols].astype(F32)
        for a in range(n_chunks):
            acc = kpad[pl.ds(8 + a * CHUNK, CHUNK), :] * taps[0:1, :]
            for j in range(1, n_taps):
                acc = acc + kpad[pl.ds(8 + a * CHUNK - j, CHUNK), :] * taps[j:j + 1, :]
            kv = acc * vs[c, pl.ds(a * CHUNK, CHUNK), :].astype(F32)
            kvf[pl.ds(a * CHUNK, CHUNK), :] = kv
            kvb[:, pl.ds(a * CHUNK, CHUNK)] = kv.astype(BF16)
        uspec[...] = _dot(fwd_ref[...], kvb[...])

        pltpu.make_async_copy(hs.at[c], hs.at[c], in_sems.at[2, c]).wait()
        hcat = jnp.concatenate(
            [hs[c, :, pl.ds(a * CHUNK, CHUNK)] for a in range(n_chunks)], axis=0)
        gspec[...] = _dot(fwd_ref[...], hcat, _NT)

        def freq_group(r, carry2):
            re = pl.ds(pl.multiple_of(r * 8, 8), 8)
            im = pl.ds(pl.multiple_of(CHUNK + r * 8, 8), 8)
            col = lambda a: pl.ds(a * LANES, LANES)
            g_re, g_im = [], []
            for a in range(n_chunks):
                gr, gi = gspec[re, col(a)], gspec[im, col(a)]
                if a > 0:
                    gr = gr - sgn * gspec[im, col(a - 1)]
                    gi = gi + sgn * gspec[re, col(a - 1)]
                g_re.append(gr)
                g_im.append(gi)
            for a in range(n_chunks):
                pr = pi = None
                for b in range(a + 1):
                    ur, ui = uspec[re, col(b)], uspec[im, col(b)]
                    tr = ur * g_re[a - b] - ui * g_im[a - b]
                    ti = ur * g_im[a - b] + ui * g_re[a - b]
                    pr = tr if pr is None else pr + tr
                    pi = ti if pi is None else pi + ti
                pspec[re, col(a)] = pr
                pspec[im, col(a)] = pi
            return carry2

        lax.fori_loop(0, CHUNK // 8, freq_group, 0)

        y = _dot(inv_ref[...], pspec[...].astype(BF16))
        pltpu.make_async_copy(xs.at[c], xs.at[c], in_sems.at[3, c]).wait()
        dvec = dvec_ref[:, cols].astype(F32)
        for a in range(n_chunks):
            t = pl.ds(a * CHUNK, CHUNK)
            ya = y[:, a * LANES:(a + 1) * LANES] + kvf[t, :] * dvec
            bterm[c, t, :] = xs[c, t, :].astype(F32) * ya
        return carry

    lax.fori_loop(0, n_ct, b_tile, 0)

    early = n_ct + 2
    ahead = 3
    for p in range(early, early + ahead):
        start_weights(p)

    def w_pair(p, carry):
        @pl.when((p >= early) & (p + ahead < n_pairs))
        def _():
            start_weights(p + ahead)

        for which in range(3):
            pltpu.make_async_copy(
                wraw.at[which, p], wraw.at[which, p], w_sems.at[which, p]).wait()
            wqkv[p, which] = pltpu.bitcast(wraw[which, p].T, jnp.uint32)
        pltpu.make_async_copy(wraw.at[3, p], wraw.at[3, p], w_sems.at[3, p]).wait()
        wo[p] = pltpu.bitcast(wraw[3, p], jnp.uint32)
        return carry

    lax.fori_loop(0, n_pairs, w_pair, 0)

    lane = lax.broadcasted_iota(jnp.int32, (rows, LANES), 1)
    lane_lo = lane < (head_dim - LANES)
    col = lax.broadcasted_iota(jnp.int32, (rows, 2 * rows), 1)
    row = lax.broadcasted_iota(jnp.int32, (rows, 2 * rows), 0)
    first = col < rows
    key = jnp.where(first, col, col - rows)
    visible = (row < n_mem) | (row >= key)
    zeros = jnp.zeros((rows, LANES), F32)
    gate_w = gw_ref[...].astype(F32)

    def split_heads(t):
        a, b, c = t[:, :LANES], t[:, LANES:2 * LANES], t[:, 2 * LANES:]
        top = jnp.concatenate([a, jnp.where(lane_lo, b, 0.0), zeros], axis=1)
        bot = jnp.concatenate([zeros, jnp.where(lane_lo, 0.0, b), c], axis=1)
        return jnp.concatenate([top, bot], axis=0).astype(BF16)

    def softmax_pair(s):
        s = jnp.where(visible, s * scale, -1000000000.0)
        m0 = jnp.max(jnp.where(first, s, -jnp.inf), axis=1, keepdims=True)
        m1 = jnp.max(jnp.where(first, -jnp.inf, s), axis=1, keepdims=True)
        e = jnp.exp(s - jnp.where(first, m0, m1))
        l0 = jnp.sum(jnp.where(first, e, 0.0), axis=1, keepdims=True)
        l1 = jnp.sum(jnp.where(first, 0.0, e), axis=1, keepdims=True)
        return e / jnp.where(first, l0, l1)

    def step(s, mem):
        t = pl.ds(pl.multiple_of(s * seg, seg), seg)
        xt = jnp.concatenate([xs[c, t, :].astype(F32) for c in range(n_ct)], axis=1)
        h = jnp.concatenate([mem, xt], axis=0)

        def proj(p, which):
            return _dot(h, pltpu.bitcast(wqkv[p, which], BF16))

        q, k, v, prob, o = {}, {}, {}, {}, {}
        acc = None
        for op, i in _mxu_order(n_pairs):
            if op == "q":
                q[i] = proj(i, 0)
            elif op == "k":
                k[i] = split_heads(proj(i, 1))
            elif op == "v":
                v[i] = split_heads(proj(i, 2))
            elif op == "s":
                prob[i] = softmax_pair(_dot(q.pop(i), k.pop(i), _NT))
            elif op == "pv":
                o[i] = _dot(prob.pop(i), v.pop(i))
            else:
                part = _dot(o.pop(i), pltpu.bitcast(wo[i], BF16))
                acc = part if acc is None else acc + part

        gate = jax.nn.sigmoid(jnp.sum(xt * gate_w, axis=1, keepdims=True))
        b = jnp.concatenate([bterm[c, t, :] for c in range(n_ct)], axis=1)
        res = gate * acc[n_mem:, :] + (1.0 - gate) * b
        obuf[t, :] = res.astype(BF16)
        pltpu.make_async_copy(obuf.at[t, :], out_hbm.at[t, :], out_sem).start()
        return acc[:n_mem, :].astype(BF16).astype(F32)

    lax.fori_loop(0, n_seg, step, mem0_ref[...].astype(F32))
    pltpu.make_async_copy(obuf, out_hbm, out_sem).wait()


@functools.partial(jax.jit, static_argnames=("A_seg_len",))
def pallas_gated_mix__memory_aug_recurrent_mem_tr__ssm_conv_h3__prompt_kernel(
    A_x: jax.Array,
    A_mem0: jax.Array,
    A_Wq: jax.Array,
    A_Wk: jax.Array,
    A_Wv: jax.Array,
    A_Wo: jax.Array,
    A_seg_len: int,
    B_q: jax.Array,
    B_k: jax.Array,
    B_v: jax.Array,
    B_shift_k: jax.Array,
    B_ssm_k: jax.Array,
    B_ssm_D: jax.Array,
    gate_w: jax.Array,
):
    del B_q
    batch, seq, dm = A_x.shape
    _, n_heads, head_dim = A_Wq.shape
    n_mem = A_mem0.shape[1]
    n_taps = B_shift_k.shape[1]
    seg = int(A_seg_len)
    assert batch == 1 and head_dim == 192 and n_heads % 2 == 0 and dm % LANES == 0
    assert seq % seg == 0 and seq % CHUNK == 0 and seg % 16 == 0 and n_mem % 8 == 0
    assert 2 * (seg + n_mem) <= LANES and n_taps <= 8
    n_ct = dm // LANES
    n_pairs = n_heads // 2
    pw = 2 * head_dim
    n_chunks = seq // CHUNK

    as_rows = lambda w: jnp.transpose(w, (1, 2, 0)).reshape(n_heads * head_dim, dm)
    fwd, inv = _dft_matrices()

    hbm = pl.BlockSpec(memory_space=pl.ANY)
    vmem = pl.BlockSpec(memory_space=pltpu.VMEM)
    out = pl.pallas_call(
        functools.partial(_kernel, seg=seg, n_mem=n_mem, n_taps=n_taps, head_dim=head_dim),
        out_shape=jax.ShapeDtypeStruct((seq, dm), BF16),
        in_specs=[hbm] * 8 + [vmem] * 6,
        out_specs=hbm,
        scratch_shapes=[
            pltpu.VMEM((n_ct, seq, LANES), BF16),
            pltpu.VMEM((n_ct, seq, LANES), BF16),
            pltpu.VMEM((n_ct, seq, LANES), BF16),
            pltpu.VMEM((n_ct, LANES, seq), BF16),
            pltpu.VMEM((4, n_pairs, pw, dm), BF16),
            pltpu.VMEM((n_pairs, 3, dm // 2, pw), jnp.uint32),
            pltpu.VMEM((n_pairs, pw // 2, dm), jnp.uint32),
            pltpu.VMEM((seq + 8, LANES), F32),
            pltpu.VMEM((seq, LANES), F32),
            pltpu.VMEM((CHUNK, n_chunks * LANES), BF16),
            pltpu.VMEM((2 * CHUNK, n_chunks * LANES), F32),
            pltpu.VMEM((2 * CHUNK, n_chunks * LANES), F32),
            pltpu.VMEM((2 * CHUNK, n_chunks * LANES), F32),
            pltpu.VMEM((n_ct, seq, LANES), F32),
            pltpu.VMEM((seq, dm), BF16),
            pltpu.SemaphoreType.DMA((4, n_ct)),
            pltpu.SemaphoreType.DMA((4, n_pairs)),
            pltpu.SemaphoreType.DMA,
        ],
        compiler_params=pltpu.CompilerParams(vmem_limit_bytes=110 * 1024 * 1024),
        name="gated_mix_rmt_h3",
    )(
        A_x.reshape(seq, dm), B_k.reshape(seq, dm), B_v.reshape(seq, dm), B_ssm_k,
        as_rows(A_Wq), as_rows(A_Wk), as_rows(A_Wv), A_Wo.reshape(n_heads * head_dim, dm),
        A_mem0.reshape(n_mem, dm), B_shift_k.T, B_ssm_D.reshape(1, dm), gate_w.reshape(1, dm),
        fwd, inv,
    )
    return out.reshape(batch, seq, dm)
```

```python
import functools

import jax
import jax.numpy as jnp
import numpy as np
from jax import lax
from jax.experimental import pallas as pl
from jax.experimental.pallas import tpu as pltpu

F32 = jnp.float32
BF16 = jnp.bfloat16
LANES = 128
SUBLANES = 8
CHUNK = 128
Q_SLOTS = 4
KVO_SLOTS = 8
PRE_ROWS = 128
PACE_START = 8
PACE_TERMS = 4

_NN = (((1,), (0,)), ((), ()))
_NT = (((1,), (1,)), ((), ()))


def _dot(a, b, dims=_NN):
    return lax.dot_general(a, b, dims, preferred_element_type=F32)


def _dft_matrices():
    k = np.arange(CHUNK, dtype=np.float64)[:, None]
    n = np.arange(CHUNK, dtype=np.float64)[None, :]
    theta = np.pi * (2.0 * k + 1.0) * n / (2.0 * CHUNK)
    fwd = np.concatenate([np.cos(theta), -np.sin(theta)], axis=0)
    inv = fwd.reshape(2, CHUNK, CHUNK).transpose(2, 1, 0).reshape(CHUNK, 2 * CHUNK) / CHUNK
    return np.asarray(fwd, dtype=BF16), np.asarray(inv, dtype=BF16)


def _mxu_order(n, lag=6):
    order = []
    for i in range(n):
        order += [("a", i), ("pv", i - 2), ("s", i - 1), ("b", i), ("c", i), ("o", i - lag)]
    held = [("o", i) for i in range(n - lag, n)]
    order += held[:1] + [("pv", n - 2), ("s", n - 1)] + held[1:-2] + [("pv", n - 1)] + held[-2:]
    return [(op, i) for op, i in order if i >= 0]


def _aligned(start, size):
    return pl.ds(pl.multiple_of(start, size), size)


def _kernel(
    x_hbm, k_hbm, v_hbm, h_hbm, wq_hbm, wk_hbm, wv_hbm, wo_hbm,
    mem0_ref, shift_ref, dvec_ref, gw_ref, fwd_ref, inv_ref,
    out_hbm,
    xs, ks, vs, hs, w_raw, wqkv, wo, kpad, kvb, dvec, uspec, gspec, pspec, qring, obuf, zero_ref,
    b_sems, x_sems, w_sems, out_sem,
    *, seg, n_mem, n_taps, head_dim,
):
    seq, dm = xs.shape
    n_ct = dm // LANES
    n_pairs = wo.shape[0]
    pw = 2 * head_dim
    n_seg = seq // seg
    n_chunks = seq // CHUNK
    rows = n_mem + seg
    scale = head_dim ** (-0.5)
    lead = seq // 2
    q_new = seg // 2
    ring = qring.shape[1]
    kvo_lag = n_ct

    def b_copy(which, c):
        cols = _aligned(c * LANES, LANES)
        src = (k_hbm.at[:, cols], v_hbm.at[:, cols], h_hbm.at[cols, :])[which]
        return pltpu.make_async_copy(src, (ks, vs, hs)[which].at[c], b_sems.at[which, c])

    def x_copy(half):
        t = pl.ds(half * lead, lead)
        return pltpu.make_async_copy(x_hbm.at[t, :], xs.at[t, :], x_sems.at[half])

    def w_slot(which, p):
        if which == 0:
            return p % Q_SLOTS
        return Q_SLOTS + (which - 1) * KVO_SLOTS + p % KVO_SLOTS

    def w_copy(which, p):
        src = (wq_hbm, wk_hbm, wv_hbm, wo_hbm)[which]
        return pltpu.make_async_copy(
            src.at[_aligned(p * pw, pw), :], w_raw.at[w_slot(which, p)], w_sems.at[which, p])

    def start_b(c):
        for which in range(3):
            b_copy(which, c).start()

    def start_kvo(p):
        for which in range(1, 4):
            w_copy(which, p).start()

    def wait_kvo(p):
        for which in range(1, 4):
            w_copy(which, p).wait()

    start_b(0)
    x_copy(0).start()
    w_copy(0, 0).start()

    kpad[pl.ds(0, SUBLANES), :] = jnp.zeros((SUBLANES, LANES), F32)

    sub = lax.broadcasted_iota(jnp.int32, (CHUNK, LANES), 0)
    sgn = jnp.where((sub & 1) == 0, 1.0, -1.0).astype(F32)
    dvec[pl.ds(0, n_ct), :] = dvec_ref[...].astype(F32)
    for a in range(n_chunks):
        zero_ref[a] = 0

    def forward_tile(c):
        for which in range(3):
            b_copy(which, c).wait()

        @pl.when(c == 0)
        def _():
            w_copy(0, 1).start()
            start_kvo(0)

        @pl.when(c + 1 < n_ct)
        def _():
            start_b(c + 1)

        kpad[pl.ds(SUBLANES, seq), :] = ks[c].astype(F32)
        taps = shift_ref[:, _aligned(c * LANES, LANES)].astype(F32)
        for a in range(n_chunks):
            acc = kpad[pl.ds(SUBLANES + a * CHUNK, CHUNK), :] * taps[0:1, :]
            for j in range(1, n_taps):
                acc = acc + kpad[pl.ds(SUBLANES + a * CHUNK - j, CHUNK), :] * taps[j:j + 1, :]
            kv = acc * vs[c, pl.ds(a * CHUNK, CHUNK), :].astype(F32)
            kvb[:, pl.ds(a * LANES, LANES)] = kv.astype(BF16)
        hcat = jnp.concatenate(
            [hs[c, :, pl.ds(a * CHUNK, CHUNK)] for a in range(n_chunks)], axis=0)
        g = _dot(fwd_ref[...], hcat, _NT)
        u = _dot(fwd_ref[...], kvb[...])
        part = lambda m, a, half: m[half * CHUNK:(half + 1) * CHUNK, a * LANES:(a + 1) * LANES]
        for a in range(n_chunks):
            g_re, g_im = part(g, a, 0), part(g, a, 1)
            if a == 0:
                g_re = g_re + dvec[pl.ds(c, 1), :]
            else:
                g_re, g_im = g_re - sgn * part(g, a - 1, 1), g_im + sgn * part(g, a - 1, 0)
            gspec[c, pl.ds(2 * a * CHUNK, CHUNK), :] = g_re
            gspec[c, pl.ds((2 * a + 1) * CHUNK, CHUNK), :] = g_im
            uspec[c, pl.ds(2 * a * CHUNK, 2 * CHUNK), :] = u[:, a * LANES:(a + 1) * LANES]

    def mix_chunks(c, r):
        re = lambda j: _aligned(2 * j * CHUNK + r * SUBLANES, SUBLANES)
        im = lambda j: _aligned((2 * j + 1) * CHUNK + r * SUBLANES, SUBLANES)
        g = [(gspec[c, re(j), :], gspec[c, im(j), :]) for j in range(n_chunks)]
        done = []
        for a in range(n_chunks):
            pr = pi = None
            for b in range(a + 1):
                ur, ui = uspec[c, re(b), :], uspec[c, im(b), :]
                gr, gi = g[a - b]
                tr, ti = ur * gr - ui * gi, ur * gi + ui * gr
                pr = tr if pr is None else pr + tr
                pi = ti if pi is None else pi + ti
                if b % PACE_TERMS == PACE_TERMS - 1 and b + 2 <= a:
                    done.append(
                        (PACE_TERMS, pltpu.bitcast(pr, jnp.int32) | pltpu.bitcast(pi, jnp.int32)))
            packed = pltpu.pack_elementwise([pr, pi], packed_dtype=BF16)
            pspec[c, _aligned(a * CHUNK + r * SUBLANES, SUBLANES), :] = packed
            done.append((a + 1 - max(a - 1, 0) // PACE_TERMS * PACE_TERMS, packed))
        return done

    def relayout(which, block, p):
        if which == 3:
            wo[p] = pltpu.bitcast(block, jnp.int32)
            return []
        bits = pltpu.bitcast(block.T, jnp.int32)
        wqkv[p, which] = bits
        return [
            (1, bits[r:r + SUBLANES, c:c + LANES])
            for r in range(0, dm // 2, LANES // 2) for c in range(0, pw, LANES)]

    def pair_prologue(p, carry):
        w_copy(0, p).wait()

        @pl.when(p == 0)
        def _():
            x_copy(0).wait()

        @pl.when(p >= kvo_lag)
        def _():
            wait_kvo(p - kvo_lag)

        @pl.when(p + 2 < n_pairs)
        def _():
            w_copy(0, p + 2).start()

        @pl.when(p + 1 < n_pairs)
        def _():
            start_kvo(p + 1)

        @pl.when(p + 2 == n_pairs)
        def _():
            x_copy(1).start()

        n_blocks = lead // PRE_ROWS
        tiles = (pw // LANES) * n_ct
        mixes = []
        for j in range(n_ct):
            group = p * n_ct + j
            mixes += mix_chunks(group // n_pairs, group % n_pairs)
        moves = relayout(0, w_raw[w_slot(0, p)], p)
        for which in range(1, 4):
            ready = p >= kvo_lag
            late = jnp.where(ready, p - kvo_lag, p)
            slot = jnp.where(ready, w_slot(which, late), w_slot(0, p))
            moves += relayout(which, w_raw[slot], late)
        pace = {}
        for work in (mixes, moves):
            total, spent = sum(cost for cost, _ in work), 0
            for cost, value in work:
                spent += cost
                slot = PACE_START + (n_blocks * tiles - 1 - PACE_START) * spent // total
                pace[slot] = pace[slot] | value if slot in pace else value
        w_bits = pltpu.bitcast(w_raw[w_slot(0, p)], jnp.int32)
        zero = zero_ref[0]
        for i in range(n_blocks):
            grid = []
            for n in range(pw // LANES):
                band = []
                for k in range(n_ct):
                    tile = w_bits[n * LANES // 2:(n + 1) * LANES // 2, k * LANES:(k + 1) * LANES]
                    slot = i * tiles + n * n_ct + k
                    if slot in pace:
                        head = tile[:SUBLANES, :] | (pace[slot] & zero)
                        tile = jnp.concatenate([head, tile[SUBLANES:, :]], axis=0)
                    band.append(tile)
                grid.append(jnp.concatenate(band, axis=1))
            w = pltpu.bitcast(jnp.concatenate(grid, axis=0), BF16)
            t = pl.ds(i * PRE_ROWS, PRE_ROWS)
            qring[p, t, :] = _dot(xs[t, :], w, _NT)
        return carry

    def tile_prologue(c, carry):
        first = lambda c: (c * n_pairs) // n_ct
        forward_tile(c)
        return lax.fori_loop(first(c), first(c + 1), pair_prologue, carry)

    lax.fori_loop(0, n_ct, tile_prologue, 0)
    x_copy(1).wait()

    def inverse_tile(c, carry):
        late = n_pairs - kvo_lag + c
        wait_kvo(late)
        spec = jnp.concatenate(
            [pltpu.bitcast(pspec[c, pl.ds(a * CHUNK, CHUNK), :], BF16) for a in range(n_chunks)],
            axis=1)
        y = _dot(inv_ref[...], spec)
        cols = _aligned(c * LANES, LANES)
        for a in range(n_chunks):
            t = pl.ds(a * CHUNK, CHUNK)
            gspec[c, t, :] = xs[t, cols].astype(F32) * y[:, a * LANES:(a + 1) * LANES]
        for which in range(1, 4):
            relayout(which, w_raw[w_slot(which, late)], late)
        return carry

    lax.fori_loop(0, n_ct, inverse_tile, 0)

    lane = lax.broadcasted_iota(jnp.int32, (rows, LANES), 1)
    lane_lo = lane < (head_dim - LANES)
    col = lax.broadcasted_iota(jnp.int32, (rows, 2 * rows), 1)
    row = lax.broadcasted_iota(jnp.int32, (rows, 2 * rows), 0)
    first = col < rows
    key = jnp.where(first, col, col - rows)
    visible = (row < n_mem) | (row >= key)
    zeros = jnp.zeros((rows, LANES), F32)
    gate_w = gw_ref[...].astype(F32)
    gate_w = jnp.concatenate([gate_w[c:c + 1, :] for c in range(n_ct)], axis=1)

    def split_heads(a, b, c):
        top = jnp.concatenate([a, jnp.where(lane_lo, b, 0.0), zeros], axis=1)
        bot = jnp.concatenate([zeros, jnp.where(lane_lo, 0.0, b), c], axis=1)
        return jnp.concatenate([top, bot], axis=0).astype(BF16)

    def softmax_pair(s):
        s = jnp.where(visible, s * scale, -1000000000.0)
        m0 = jnp.max(jnp.where(first, s, -jnp.inf), axis=1, keepdims=True)
        m1 = jnp.max(jnp.where(first, -jnp.inf, s), axis=1, keepdims=True)
        e = jnp.exp(s - jnp.where(first, m0, m1))
        l0 = jnp.sum(jnp.where(first, e, 0.0), axis=1, keepdims=True)
        l1 = jnp.sum(jnp.where(first, 0.0, e), axis=1, keepdims=True)
        return e / jnp.where(first, l0, l1)

    def step(s, carry):
        mem, q_put, q_get = carry
        t = _aligned(s * seg, seg)
        xt = xs[t, :].astype(F32)
        h = jnp.concatenate([mem, xt], axis=0)
        hq = jnp.concatenate(
            [mem, xs[_aligned(lead + s * q_new, q_new), :].astype(F32)], axis=0)

        def project(p, j):
            w = lambda which: pltpu.bitcast(wqkv[p, which, :, pl.ds(j * LANES, LANES)], BF16)
            new = _dot(hq, w(0))
            cols = pl.ds(j * LANES, LANES)
            qring[p, _aligned(q_put, q_new), cols] = new[n_mem:, :]
            q = jnp.concatenate([new[:n_mem, :], qring[p, _aligned(q_get, seg), cols]], axis=0)
            return q, _dot(h, w(1)), _dot(h, w(2))

        q, k, v, prob, o, tiles = {}, {}, {}, {}, {}, []
        acc = None
        for op, i in _mxu_order(n_pairs):
            if op in "abc":
                tiles.append(project(i, len(tiles)))
                if op == "c":
                    q[i] = jnp.concatenate([t3[0] for t3 in tiles], axis=1)
                    k[i] = split_heads(*[t3[1] for t3 in tiles])
                    v[i] = split_heads(*[t3[2] for t3 in tiles])
                    tiles = []
            elif op == "s":
                prob[i] = softmax_pair(_dot(q.pop(i), k.pop(i), _NT))
            elif op == "pv":
                o[i] = _dot(prob.pop(i), v.pop(i))
            else:
                part = _dot(o.pop(i), pltpu.bitcast(wo[i], BF16))
                acc = part if acc is None else acc + part

        gate = jax.nn.sigmoid(jnp.sum(xt * gate_w, axis=1, keepdims=True))
        b = jnp.concatenate([gspec[c, t, :] for c in range(n_ct)], axis=1)
        res = gate * acc[n_mem:, :] + (1.0 - gate) * b
        obuf[t, :] = res.astype(BF16)
        pltpu.make_async_copy(obuf.at[t, :], out_hbm.at[t, :], out_sem).start()
        wrap = lambda pos: jnp.where(pos >= ring, pos - ring, pos)
        return acc[:n_mem, :].astype(BF16).astype(F32), wrap(q_put + q_new), wrap(q_get + seg)

    lax.fori_loop(
        0, n_seg, step, (mem0_ref[...].astype(F32), jnp.int32(lead), jnp.int32(0)))
    pltpu.make_async_copy(obuf, out_hbm, out_sem).wait()


@functools.partial(jax.jit, static_argnames=("A_seg_len",))
def pallas_gated_mix__memory_aug_recurrent_mem_tr__ssm_conv_h3__prompt_kernel(
    A_x: jax.Array,
    A_mem0: jax.Array,
    A_Wq: jax.Array,
    A_Wk: jax.Array,
    A_Wv: jax.Array,
    A_Wo: jax.Array,
    A_seg_len: int,
    B_q: jax.Array,
    B_k: jax.Array,
    B_v: jax.Array,
    B_shift_k: jax.Array,
    B_ssm_k: jax.Array,
    B_ssm_D: jax.Array,
    gate_w: jax.Array,
):
    del B_q
    batch, seq, dm = A_x.shape
    _, n_heads, head_dim = A_Wq.shape
    n_mem = A_mem0.shape[1]
    n_taps = B_shift_k.shape[1]
    seg = int(A_seg_len)
    n_ct = dm // LANES
    n_pairs = n_heads // 2
    pw = 2 * head_dim
    n_chunks = seq // CHUNK
    assert batch == 1 and 2 * head_dim == 3 * LANES and dm % LANES == 0
    assert n_heads == 2 * (CHUNK // SUBLANES) and n_ct + 2 <= KVO_SLOTS
    assert seq % seg == 0 and seq % (2 * PRE_ROWS) == 0 and seg % 32 == 0
    assert n_mem % SUBLANES == 0 and 2 * (seg + n_mem) <= LANES and n_taps <= SUBLANES

    as_rows = lambda w: jnp.transpose(w, (1, 2, 0)).reshape(n_heads * head_dim, dm)
    fwd, inv = _dft_matrices()

    hbm = pl.BlockSpec(memory_space=pl.ANY)
    vmem = pl.BlockSpec(memory_space=pltpu.VMEM)
    out = pl.pallas_call(
        functools.partial(_kernel, seg=seg, n_mem=n_mem, n_taps=n_taps, head_dim=head_dim),
        out_shape=jax.ShapeDtypeStruct((seq, dm), BF16),
        in_specs=[hbm] * 8 + [vmem] * 6,
        out_specs=hbm,
        scratch_shapes=[
            pltpu.VMEM((seq, dm), BF16),
            pltpu.VMEM((n_ct, seq, LANES), BF16),
            pltpu.VMEM((n_ct, seq, LANES), BF16),
            pltpu.VMEM((n_ct, LANES, seq), BF16),
            pltpu.VMEM((Q_SLOTS + 3 * KVO_SLOTS, pw, dm), BF16),
            pltpu.VMEM((n_pairs, 3, dm // 2, pw), jnp.int32),
            pltpu.VMEM((n_pairs, pw // 2, dm), jnp.int32),
            pltpu.VMEM((seq + SUBLANES, LANES), F32),
            pltpu.VMEM((CHUNK, n_chunks * LANES), BF16),
            pltpu.VMEM((SUBLANES, LANES), F32),
            pltpu.VMEM((n_ct, 2 * seq, LANES), F32),
            pltpu.VMEM((n_ct, 2 * seq, LANES), F32),
            pltpu.VMEM((n_ct, seq, LANES), jnp.int32),
            pltpu.VMEM((n_pairs, seq // 2 + seg, pw), F32),
            pltpu.VMEM((seq, dm), BF16),
            pltpu.SMEM((n_chunks,), jnp.int32),
            pltpu.SemaphoreType.DMA((3, n_ct)),
            pltpu.SemaphoreType.DMA((2,)),
            pltpu.SemaphoreType.DMA((4, n_pairs)),
            pltpu.SemaphoreType.DMA,
        ],
        compiler_params=pltpu.CompilerParams(
            vmem_limit_bytes=116 * 1024 * 1024, disable_bounds_checks=True),
        name="gated_mix_rmt_h3",
    )(
        A_x.reshape(seq, dm), B_k.reshape(seq, dm), B_v.reshape(seq, dm), B_ssm_k,
        as_rows(A_Wq), as_rows(A_Wk), as_rows(A_Wv), A_Wo.reshape(n_heads * head_dim, dm),
        A_mem0.reshape(n_mem, dm), B_shift_k.T,
        B_ssm_D.reshape(n_ct, LANES), gate_w.reshape(n_ct, LANES), fwd, inv,
    )
    return out.reshape(batch, seq, dm)
```

```python
import functools

import jax
import jax.numpy as jnp
import numpy as np
from jax import lax
from jax.experimental import pallas as pl
from jax.experimental.pallas import tpu as pltpu

F32 = jnp.float32
BF16 = jnp.bfloat16
I32 = jnp.int32
LANES = 128
SUBLANES = 8
CHUNK = 128
FWD_CHUNKS = 1
Q_SLOTS = 4
KVO_SLOTS = 8
PRE_ROWS = 128
PACE_START = 8
PACE_TERMS = 4
UNROLL = 4

_NN = (((1,), (0,)), ((), ()))
_NT = (((1,), (1,)), ((), ()))


def _dot(a, b, dims=_NN):
    return lax.dot_general(a, b, dims, preferred_element_type=F32)


def _aligned(start, size):
    return pl.ds(pl.multiple_of(start, size), size)


def _dft_matrices():
    k = np.arange(CHUNK, dtype=np.float64)[:, None]
    n = np.arange(CHUNK, dtype=np.float64)[None, :]
    theta = np.pi * (2.0 * k + 1.0) * n / (2.0 * CHUNK)
    parts = np.stack([np.cos(theta), -np.sin(theta)])
    fwd = parts.reshape(2 * CHUNK, CHUNK)
    inv = parts.transpose(2, 1, 0).reshape(CHUNK, 2 * CHUNK) / CHUNK
    return np.asarray(fwd, dtype=BF16), np.asarray(inv, dtype=BF16)


def _mxu_order(n, lag=6):
    order = []
    for i in range(n):
        order += [("qkv", i), ("qkv", i), ("s", i - 1), ("qkv", i), ("o", i - lag), ("pv", i - 2)]
    held = [("o", i) for i in range(n - lag, n)]
    order += held[:1] + [("pv", n - 2), ("s", n - 1)] + held[1:-2] + [("pv", n - 1)] + held[-2:]
    return [(op, i) for op, i in order if i >= 0]


def _kernel(
    x_hbm, k_hbm, v_hbm, h_hbm, wq_hbm, wk_hbm, wv_hbm, wo_hbm,
    mem0_hbm, shift_hbm, skip_hbm, gate_hbm, fwd_hbm, inv_hbm,
    out_hbm,
    mem0_ref, shift_ref, skip_ref, gate_ref, fwd_ref, inv_ref,
    xs, ks, vs, hs, w_raw, wqkv, wo, skip, uspec, gspec, pspec, qring, obuf, zero_ref,
    small_sem, b_sems, x_sems, q_sems, kvo_sems, out_sem,
    *, seg, n_mem, n_taps, head_dim,
):
    seq, dm = xs.shape
    n_ct = dm // LANES
    n_pairs = wo.shape[0]
    pw = 2 * head_dim
    n_seg = seq // seg
    n_chunks = seq // CHUNK
    rows = n_mem + seg
    scale = head_dim ** (-0.5)
    lead = seq // 2
    q_new = seg // 2
    ring = qring.shape[1]
    kvo_lag = n_ct

    small = [
        pltpu.make_async_copy(src, dst, small_sem)
        for src, dst in (
            (fwd_hbm, fwd_ref), (shift_hbm, shift_ref), (skip_hbm, skip_ref),
            (inv_hbm, inv_ref), (mem0_hbm, mem0_ref), (gate_hbm, gate_ref))]

    def b_copies(c):
        cols = _aligned(c * LANES, LANES)
        return [
            pltpu.make_async_copy(src, dst.at[c % 2], b_sems.at[c % 2])
            for src, dst in (
                (h_hbm.at[cols, :], hs), (k_hbm.at[:, cols], ks), (v_hbm.at[:, cols], vs))]

    def x_copy(half):
        t = pl.ds(half * lead, lead)
        return pltpu.make_async_copy(x_hbm.at[t, :], xs.at[t, :], x_sems.at[half])

    def w_slot(which, p):
        if which == 0:
            return p % Q_SLOTS
        return Q_SLOTS + (which - 1) * KVO_SLOTS + p % KVO_SLOTS

    def q_copy(p):
        return pltpu.make_async_copy(
            wq_hbm.at[_aligned(p * pw, pw), :], w_raw.at[w_slot(0, p)], q_sems.at[p % Q_SLOTS])

    def kvo_copies(p):
        return [
            pltpu.make_async_copy(
                src.at[_aligned(p * pw, pw), :], w_raw.at[w_slot(which, p)],
                kvo_sems.at[p % KVO_SLOTS])
            for which, src in ((1, wk_hbm), (2, wv_hbm), (3, wo_hbm))]

    def start(copies):
        for copy in copies:
            copy.start()

    def wait(copies):
        for copy in copies:
            copy.wait()

    start(small)
    start(b_copies(0))
    x_copy(0).start()
    q_copy(0).start()
    zero_ref[0] = 0
    wait(small)

    bins = lax.broadcasted_iota(I32, (CHUNK, LANES), 0)
    sign = jnp.where((bins & 1) == 0, 1.0, -1.0).astype(F32)
    skip[pl.ds(0, n_ct), :] = skip_ref[...].astype(F32)

    def forward_tile(c):
        wait(b_copies(c))

        @pl.when(c == 0)
        def _():
            q_copy(1).start()
            start(kvo_copies(0))

        @pl.when(c + 1 < n_ct)
        def _():
            start(b_copies(c + 1))

        taps = shift_ref[:, _aligned(c * LANES, LANES)].astype(F32)
        before = jnp.zeros((SUBLANES, LANES), F32)
        last = None
        for a0 in range(0, n_chunks, FWD_CHUNKS):
            group = range(a0, a0 + FWD_CHUNKS)
            kv = []
            for a in group:
                t = pl.ds(a * CHUNK, CHUNK)
                keys = ks[c % 2, t, :].astype(F32)
                past = jnp.concatenate([before, keys], axis=0)
                before = keys[CHUNK - SUBLANES:, :]
                acc = keys * taps[0:1, :]
                for j in range(1, n_taps):
                    acc = acc + past[SUBLANES - j:SUBLANES - j + CHUNK, :] * taps[j:j + 1, :]
                kv.append((acc * vs[c % 2, t, :].astype(F32)).astype(BF16))
            filt = jnp.concatenate(
                [hs[c % 2, :, pl.ds(a * CHUNK, CHUNK)] for a in group], axis=0)
            g = _dot(fwd_ref[...], filt, _NT)
            u = _dot(fwd_ref[...], jnp.concatenate(kv, axis=1))
            for a in group:
                cols = slice((a - a0) * LANES, (a - a0 + 1) * LANES)
                g_re, g_im = g[:CHUNK, cols], g[CHUNK:, cols]
                if last is None:
                    out = g_re + skip[pl.ds(c, 1), :], g_im
                else:
                    out = g_re - sign * last[1], g_im + sign * last[0]
                last = g_re, g_im
                gspec[c % 2, pl.ds(2 * a * CHUNK, CHUNK), :] = out[0]
                gspec[c % 2, pl.ds((2 * a + 1) * CHUNK, CHUNK), :] = out[1]
                uspec[c % 2, pl.ds(2 * a * CHUNK, 2 * CHUNK), :] = u[:, cols]

    def mix_chunks(c, r):
        re = lambda j: _aligned(2 * j * CHUNK + r * SUBLANES, SUBLANES)
        im = lambda j: _aligned((2 * j + 1) * CHUNK + r * SUBLANES, SUBLANES)
        g = [(gspec[c % 2, re(j), :], gspec[c % 2, im(j), :]) for j in range(n_chunks)]
        done = []
        for a in range(n_chunks):
            pr = pi = None
            paced = 0
            for b in range(a + 1):
                ur, ui = uspec[c % 2, re(b), :], uspec[c % 2, im(b), :]
                gr, gi = g[a - b]
                tr, ti = ur * gr - ui * gi, ur * gi + ui * gr
                pr = tr if pr is None else pr + tr
                pi = ti if pi is None else pi + ti
                if b + 1 - paced == PACE_TERMS and b + 2 <= a:
                    done.append((PACE_TERMS, pltpu.bitcast(pr, I32) | pltpu.bitcast(pi, I32)))
                    paced = b + 1
            packed = pltpu.pack_elementwise([pr, pi], packed_dtype=BF16)
            pspec[c, _aligned(a * CHUNK + r * SUBLANES, SUBLANES), :] = packed
            done.append((a + 1 - paced, packed))
        return done

    def relayout(which, block, p):
        if which == 3:
            wo[p] = pltpu.bitcast(block, I32)
        else:
            wqkv[p, which] = pltpu.bitcast(block.T, I32)

    def pair_prologue(p, carry):
        q_copy(p).wait()

        @pl.when(p == 0)
        def _():
            x_copy(0).wait()

        @pl.when(p >= kvo_lag)
        def _():
            wait(kvo_copies(p - kvo_lag))

        @pl.when(p + 2 < n_pairs)
        def _():
            q_copy(p + 2).start()

        @pl.when(p + 1 < n_pairs)
        def _():
            start(kvo_copies(p + 1))

        @pl.when(p + 2 == n_pairs)
        def _():
            x_copy(1).start()

        work = []
        for j in range(n_ct):
            group = p * n_ct + j
            work += mix_chunks(group // n_pairs, group % n_pairs)

        relayout(0, w_raw[w_slot(0, p)], p)
        ready = p >= kvo_lag
        late = jnp.where(ready, p - kvo_lag, p)
        for which in range(1, 4):
            relayout(which, w_raw[jnp.where(ready, w_slot(which, late), w_slot(0, p))], late)

        n_blocks = lead // PRE_ROWS
        tiles = (pw // LANES) * n_ct
        total, spent, pace = sum(cost for cost, _ in work), 0, {}
        for cost, value in work:
            spent += cost
            slot = PACE_START + (n_blocks * tiles - 1 - PACE_START) * spent // total
            pace[slot] = pace[slot] | value if slot in pace else value
        w_bits = pltpu.bitcast(w_raw[w_slot(0, p)], I32)
        zero = zero_ref[0]
        for i in range(n_blocks):
            bands = []
            for n in range(pw // LANES):
                band = []
                for c in range(n_ct):
                    tile = w_bits[n * LANES // 2:(n + 1) * LANES // 2, c * LANES:(c + 1) * LANES]
                    slot = i * tiles + n * n_ct + c
                    if slot in pace:
                        head = tile[:SUBLANES, :] | (pace[slot] & zero)
                        tile = jnp.concatenate([head, tile[SUBLANES:, :]], axis=0)
                    band.append(tile)
                bands.append(jnp.concatenate(band, axis=1))
            w = pltpu.bitcast(jnp.concatenate(bands, axis=0), BF16)
            t = pl.ds(i * PRE_ROWS, PRE_ROWS)
            qring[p, t, :] = _dot(xs[t, :], w, _NT)
        return carry

    def tile_prologue(c, carry):
        first = lambda c: (c * n_pairs) // n_ct
        forward_tile(c)
        return lax.fori_loop(first(c), first(c + 1), pair_prologue, carry)

    lax.fori_loop(0, n_ct, tile_prologue, 0)
    x_copy(1).wait()

    def inverse_tile(c, carry):
        late = n_pairs - kvo_lag + c
        wait(kvo_copies(late))
        spec = jnp.concatenate(
            [pltpu.bitcast(pspec[c, pl.ds(a * CHUNK, CHUNK), :], BF16) for a in range(n_chunks)],
            axis=1)
        y = _dot(inv_ref[...], spec)
        for a in range(n_chunks):
            t = pl.ds(a * CHUNK, CHUNK)
            pspec[c, t, :] = pltpu.bitcast(
                xs[t, _aligned(c * LANES, LANES)].astype(F32) * y[:, a * LANES:(a + 1) * LANES],
                I32)
        for which in range(1, 4):
            relayout(which, w_raw[w_slot(which, late)], late)
        return carry

    lax.fori_loop(0, n_ct, inverse_tile, 0)

    lane_lo = lax.broadcasted_iota(I32, (rows, LANES), 1) < (head_dim - LANES)
    col = lax.broadcasted_iota(I32, (rows, 2 * rows), 1)
    row = lax.broadcasted_iota(I32, (rows, 2 * rows), 0)
    head0 = col < rows
    key = jnp.where(head0, col, col - rows)
    visible = (row < n_mem) | (key >= seg) | (row - n_mem >= key)
    zeros = jnp.zeros((rows, LANES), F32)
    gate_w = gate_ref[...].astype(F32)
    gate_w = jnp.concatenate([gate_w[c:c + 1, :] for c in range(n_ct)], axis=1)

    def split_heads(a, b, c):
        top = jnp.concatenate([a, jnp.where(lane_lo, b, 0.0), zeros], axis=1)
        bottom = jnp.concatenate([zeros, jnp.where(lane_lo, 0.0, b), c], axis=1)
        return jnp.concatenate([top, bottom], axis=0).astype(BF16)

    def softmax_pair(s):
        s = jnp.where(visible, s * scale, -1000000000.0)
        m0 = jnp.max(jnp.where(head0, s, -jnp.inf), axis=1, keepdims=True)
        m1 = jnp.max(jnp.where(head0, -jnp.inf, s), axis=1, keepdims=True)
        e = jnp.exp(s - jnp.where(head0, m0, m1))
        l0 = jnp.sum(jnp.where(head0, e, 0.0), axis=1, keepdims=True)
        l1 = jnp.sum(jnp.where(head0, 0.0, e), axis=1, keepdims=True)
        return e / jnp.where(head0, l0, l1)

    def step(s, carry):
        mem, q_put, q_get = carry
        t = _aligned(s * seg, seg)
        xt = xs[t, :].astype(F32)
        h = jnp.concatenate([xt, mem], axis=0)
        hq = jnp.concatenate(
            [xs[_aligned(lead + s * q_new, q_new), :].astype(F32), mem], axis=0)

        def project(p, j):
            cols = pl.ds(j * LANES, LANES)
            w = lambda which: pltpu.bitcast(wqkv[p, which, :, cols], BF16)
            new = _dot(hq, w(0))
            qring[p, _aligned(q_put, q_new), cols] = new[:q_new, :]
            q = jnp.concatenate([new[q_new:, :], qring[p, _aligned(q_get, seg), cols]], axis=0)
            return q, _dot(h, w(1)), _dot(h, w(2))

        q, k, v, prob, o, parts = {}, {}, {}, {}, {}, []
        acc = None
        for op, i in _mxu_order(n_pairs):
            if op == "qkv":
                parts.append(project(i, len(parts)))
                if len(parts) == pw // LANES:
                    q[i] = jnp.concatenate([part[0] for part in parts], axis=1)
                    k[i] = split_heads(*[part[1] for part in parts])
                    v[i] = split_heads(*[part[2] for part in parts])
                    parts = []
            elif op == "s":
                prob[i] = softmax_pair(_dot(q.pop(i), k.pop(i), _NT))
            elif op == "pv":
                o[i] = _dot(prob.pop(i), v.pop(i))
            else:
                part = _dot(o.pop(i), pltpu.bitcast(wo[i], BF16))
                acc = part if acc is None else acc + part

        gate = jax.nn.sigmoid(jnp.sum(xt * gate_w, axis=1, keepdims=True))
        b = jnp.concatenate([pspec[c, t, :] for c in range(n_ct)], axis=1)
        res = gate * acc[n_mem:, :] + (1.0 - gate) * pltpu.bitcast(b, F32)
        obuf[t, :] = res.astype(BF16)
        pltpu.make_async_copy(obuf.at[t, :], out_hbm.at[t, :], out_sem).start()
        wrap = lambda pos: jnp.where(pos >= ring, pos - ring, pos)
        return acc[:n_mem, :].astype(BF16).astype(F32), wrap(q_put + q_new), wrap(q_get + seg)

    lax.fori_loop(
        0, n_seg, step, (mem0_ref[...].astype(F32), jnp.int32(lead), jnp.int32(0)),
        unroll=UNROLL)
    pltpu.make_async_copy(obuf, out_hbm, out_sem).wait()


@functools.partial(jax.jit, static_argnames=("A_seg_len",))
def pallas_gated_mix__memory_aug_recurrent_mem_tr__ssm_conv_h3__prompt_kernel(
    A_x: jax.Array,
    A_mem0: jax.Array,
    A_Wq: jax.Array,
    A_Wk: jax.Array,
    A_Wv: jax.Array,
    A_Wo: jax.Array,
    A_seg_len: int,
    B_q: jax.Array,
    B_k: jax.Array,
    B_v: jax.Array,
    B_shift_k: jax.Array,
    B_ssm_k: jax.Array,
    B_ssm_D: jax.Array,
    gate_w: jax.Array,
):
    del B_q
    batch, seq, dm = A_x.shape
    _, n_heads, head_dim = A_Wq.shape
    n_mem = A_mem0.shape[1]
    n_taps = B_shift_k.shape[1]
    seg = int(A_seg_len)
    n_ct = dm // LANES
    n_pairs = n_heads // 2
    pw = 2 * head_dim
    assert batch == 1 and 2 * head_dim == 3 * LANES and dm % LANES == 0
    assert n_pairs == CHUNK // SUBLANES and n_ct + 2 <= KVO_SLOTS
    assert seq % (UNROLL * seg) == 0 and seq % (2 * PRE_ROWS) == 0 and seg % 32 == 0
    assert n_mem % SUBLANES == 0 and 2 * (seg + n_mem) <= LANES and n_taps <= SUBLANES

    as_rows = lambda w: jnp.transpose(w, (1, 2, 0)).reshape(n_heads * head_dim, dm)
    fwd, inv = _dft_matrices()
    small = (
        A_mem0.reshape(n_mem, dm), B_shift_k.T, B_ssm_D.reshape(n_ct, LANES),
        gate_w.reshape(n_ct, LANES), fwd, inv)

    hbm = pl.BlockSpec(memory_space=pl.ANY)
    out = pl.pallas_call(
        functools.partial(_kernel, seg=seg, n_mem=n_mem, n_taps=n_taps, head_dim=head_dim),
        out_shape=jax.ShapeDtypeStruct((seq, dm), BF16),
        in_specs=[hbm] * (8 + len(small)),
        out_specs=hbm,
        scratch_shapes=[pltpu.VMEM(a.shape, BF16) for a in small] + [
            pltpu.VMEM((seq, dm), BF16),
            pltpu.VMEM((2, seq, LANES), BF16),
            pltpu.VMEM((2, seq, LANES), BF16),
            pltpu.VMEM((2, LANES, seq), BF16),
            pltpu.VMEM((Q_SLOTS + 3 * KVO_SLOTS, pw, dm), BF16),
            pltpu.VMEM((n_pairs, 3, dm // 2, pw), I32),
            pltpu.VMEM((n_pairs, pw // 2, dm), I32),
            pltpu.VMEM((SUBLANES, LANES), F32),
            pltpu.VMEM((2, 2 * seq, LANES), F32),
            pltpu.VMEM((2, 2 * seq, LANES), F32),
            pltpu.VMEM((n_ct, seq, LANES), I32),
            pltpu.VMEM((n_pairs, seq // 2 + seg, pw), F32),
            pltpu.VMEM((seq, dm), BF16),
            pltpu.SMEM((1,), I32),
            pltpu.SemaphoreType.DMA,
            pltpu.SemaphoreType.DMA((2,)),
            pltpu.SemaphoreType.DMA((2,)),
            pltpu.SemaphoreType.DMA((Q_SLOTS,)),
            pltpu.SemaphoreType.DMA((KVO_SLOTS,)),
            pltpu.SemaphoreType.DMA,
        ],
        compiler_params=pltpu.CompilerParams(
            vmem_limit_bytes=112 * 1024 * 1024, disable_bounds_checks=True),
        name="gated_mix_rmt_h3",
    )(
        A_x.reshape(seq, dm), B_k.reshape(seq, dm), B_v.reshape(seq, dm), B_ssm_k,
        as_rows(A_Wq), as_rows(A_Wk), as_rows(A_Wv), A_Wo.reshape(n_heads * head_dim, dm),
        *small,
    )
    return out.reshape(batch, seq, dm)
```

```python
import functools

import jax
import jax.numpy as jnp
import numpy as np
from jax import lax
from jax.experimental import pallas as pl
from jax.experimental.pallas import tpu as pltpu

F32 = jnp.float32
BF16 = jnp.bfloat16
I32 = jnp.int32
LANES = 128
SUBLANES = 8
CHUNK = 128
FWD_CHUNKS = 1
Q_AHEAD = 4
Q_SLOTS = Q_AHEAD + 1
KVO_SLOTS = 7
PRE_ROWS = 64
PACE_START = 16
PACE_TERMS = 3
UNROLL = 4

_NN = (((1,), (0,)), ((), ()))
_NT = (((1,), (1,)), ((), ()))


def _dot(a, b, dims=_NN):
    return lax.dot_general(a, b, dims, preferred_element_type=F32)


def _aligned(start, size):
    return pl.ds(pl.multiple_of(start, size), size)


def _dft_matrices():
    k = np.arange(CHUNK, dtype=np.float64)[:, None]
    n = np.arange(CHUNK, dtype=np.float64)[None, :]
    theta = np.pi * (2.0 * k + 1.0) * n / (2.0 * CHUNK)
    parts = np.stack([np.cos(theta), -np.sin(theta)])
    fwd = parts.reshape(2 * CHUNK, CHUNK)
    inv = parts.reshape(2, CHUNK // SUBLANES, SUBLANES, CHUNK).transpose(3, 1, 0, 2)
    inv = inv.reshape(CHUNK, 2 * CHUNK) / CHUNK
    return np.asarray(fwd, dtype=BF16), np.asarray(inv, dtype=BF16)


def _mxu_order(n, lag=6):
    order = []
    for i in range(n):
        order += [("qkv", i), ("qkv", i), ("s", i - 1), ("qkv", i), ("o", i - lag), ("pv", i - 2)]
    held = [("o", i) for i in range(n - lag, n)]
    order += held[:1] + [("pv", n - 2), ("s", n - 1)] + held[1:-2] + [("pv", n - 1)] + held[-2:]
    return [(op, i) for op, i in order if i >= 0]


def _kernel(
    x_hbm, k_hbm, v_hbm, h_hbm, wq_hbm, wk_hbm, wv_hbm, wo_hbm,
    mem0_hbm, shift_hbm, skip_hbm, gate_hbm, fwd_hbm, inv_hbm,
    out_hbm,
    mem0_ref, shift_ref, skip_ref, gate_ref, fwd_ref, inv_ref,
    xs, x_words, ks, vs, hs, w_raw, wqkv, wo, skip, uspec, gspec, pspec, qring, obuf, zero_ref,
    small_sem, b_sems, x_sems, q_sems, kvo_sems, out_sem,
    *, seg, n_mem, n_taps, head_dim,
):
    seq, dm = xs.shape
    n_ct = dm // LANES
    n_pairs = wo.shape[0]
    pw = 2 * head_dim
    n_seg = seq // seg
    n_chunks = seq // CHUNK
    rows = n_mem + seg
    scale = head_dim ** (-0.5)
    lead = seq // 2
    q_new = seg // 2
    ring = qring.shape[1]
    kvo_lag = n_ct

    small = [
        pltpu.make_async_copy(src, dst, small_sem)
        for src, dst in (
            (fwd_hbm, fwd_ref), (shift_hbm, shift_ref), (skip_hbm, skip_ref),
            (inv_hbm, inv_ref), (mem0_hbm, mem0_ref), (gate_hbm, gate_ref))]

    def b_copies(c):
        cols = _aligned(c * LANES, LANES)
        return [
            pltpu.make_async_copy(src, dst.at[c % 2], b_sems.at[c % 2])
            for src, dst in (
                (h_hbm.at[cols, :], hs), (k_hbm.at[:, cols], ks), (v_hbm.at[:, cols], vs))]

    def x_copy(half):
        t = pl.ds(half * lead, lead)
        return pltpu.make_async_copy(x_hbm.at[t, :], xs.at[t, :], x_sems.at[half])

    def w_slot(which, p):
        if which == 0:
            return p % Q_SLOTS
        return Q_SLOTS + (which - 1) * KVO_SLOTS + p % KVO_SLOTS

    def q_copy(p):
        return pltpu.make_async_copy(
            wq_hbm.at[_aligned(p * pw, pw), :], w_raw.at[w_slot(0, p)], q_sems.at[p % Q_SLOTS])

    def kvo_copies(p):
        return [
            pltpu.make_async_copy(
                src.at[_aligned(p * pw, pw), :], w_raw.at[w_slot(which, p)],
                kvo_sems.at[p % KVO_SLOTS])
            for which, src in ((1, wk_hbm), (2, wv_hbm), (3, wo_hbm))]

    def start(copies):
        for copy in copies:
            copy.start()

    def wait(copies):
        for copy in copies:
            copy.wait()

    start(small)
    start(b_copies(0))
    q_copy(0).start()
    x_copy(0).start()
    q_copy(1).start()
    zero_ref[0] = 0
    wait(small)

    bins = lax.broadcasted_iota(I32, (CHUNK, LANES), 0)
    sign = jnp.where((bins & 1) == 0, 1.0, -1.0).astype(F32)
    skip[pl.ds(0, n_ct), :] = skip_ref[...].astype(F32)

    def forward_tile(c):
        wait(b_copies(c))

        taps = shift_ref[:, _aligned(c * LANES, LANES)].astype(F32)
        before = jnp.zeros((SUBLANES, LANES), F32)
        last = None
        for a0 in range(0, n_chunks, FWD_CHUNKS):
            group = range(a0, a0 + FWD_CHUNKS)
            kv = []
            for a in group:
                t = pl.ds(a * CHUNK, CHUNK)
                keys = ks[c % 2, t, :].astype(F32)
                past = jnp.concatenate([before, keys], axis=0)
                before = keys[CHUNK - SUBLANES:, :]
                acc = keys * taps[0:1, :]
                for j in range(1, n_taps):
                    acc = acc + past[SUBLANES - j:SUBLANES - j + CHUNK, :] * taps[j:j + 1, :]
                kv.append((acc * vs[c % 2, t, :].astype(F32)).astype(BF16))
            filt = jnp.concatenate(
                [hs[c % 2, :, pl.ds(a * CHUNK, CHUNK)] for a in group], axis=0)
            g = _dot(fwd_ref[...], filt, _NT)
            u = _dot(fwd_ref[...], jnp.concatenate(kv, axis=1))
            for a in group:
                cols = slice((a - a0) * LANES, (a - a0 + 1) * LANES)
                g_re, g_im = g[:CHUNK, cols], g[CHUNK:, cols]
                if last is None:
                    out = g_re + skip[pl.ds(c, 1), :], g_im
                else:
                    out = g_re - sign * last[1], g_im + sign * last[0]
                last = g_re, g_im
                gspec[c % 2, pl.ds(2 * a * CHUNK, CHUNK), :] = out[0]
                gspec[c % 2, pl.ds((2 * a + 1) * CHUNK, CHUNK), :] = out[1]
                uspec[c % 2, pl.ds(2 * a * CHUNK, 2 * CHUNK), :] = u[:, cols]

        @pl.when(c + 1 < n_ct)
        def _():
            start(b_copies(c + 1))

    def mix_chunks(c, r):
        re = lambda j: _aligned(2 * j * CHUNK + r * SUBLANES, SUBLANES)
        im = lambda j: _aligned((2 * j + 1) * CHUNK + r * SUBLANES, SUBLANES)
        g = [(gspec[c % 2, re(j), :], gspec[c % 2, im(j), :]) for j in range(n_chunks)]
        done = []
        for a in range(n_chunks):
            pr = pi = None
            paced = 0
            for b in range(a + 1):
                ur, ui = uspec[c % 2, re(b), :], uspec[c % 2, im(b), :]
                gr, gi = g[a - b]
                tr, ti = ur * gr - ui * gi, ur * gi + ui * gr
                pr = tr if pr is None else pr + tr
                pi = ti if pi is None else pi + ti
                if b + 1 - paced == PACE_TERMS and b + 2 <= a:
                    done.append((PACE_TERMS, pltpu.bitcast(pr, I32) | pltpu.bitcast(pi, I32)))
                    paced = b + 1
            packed = pltpu.bitcast(jnp.concatenate([pr, pi], axis=0).astype(BF16), I32)
            pspec[c, _aligned(a * CHUNK + r * SUBLANES, SUBLANES), :] = packed
            done.append((a + 1 - paced, packed))
        return done

    def relayout(which, block, p):
        if which == 3:
            wo[p] = pltpu.bitcast(block, I32)
        else:
            wqkv[p, which] = pltpu.bitcast(block.T, I32)

    def pair_prologue(p, carry):
        @pl.when(p == 0)
        def _():
            q_copy(0).wait()
            relayout(0, w_raw[w_slot(0, 0)], 0)
            x_copy(0).wait()
            x_words[...] = pltpu.bitcast(xs[pl.ds(0, lead), :], I32)
            for ahead in range(2, Q_AHEAD):
                q_copy(ahead).start()

        @pl.when(p + Q_AHEAD < n_pairs)
        def _():
            q_copy(p + Q_AHEAD).start()

        start(kvo_copies(p))

        @pl.when(p + Q_AHEAD == n_pairs)
        def _():
            x_copy(1).start()

        @pl.when(p + 1 < n_pairs)
        def _():
            q_copy(p + 1).wait()

        @pl.when(p >= kvo_lag)
        def _():
            wait(kvo_copies(p - kvo_lag))

        work = []
        for j in range(n_ct):
            group = p * n_ct + j
            work += mix_chunks(group // n_pairs, group % n_pairs)

        n_blocks = lead // PRE_ROWS
        n_cols = pw // LANES
        slots = n_blocks * n_cols * n_ct
        total, spent, pace = sum(cost for cost, _ in work), 0, {}
        for cost, value in work:
            spent += cost
            slot = PACE_START + (slots - 1 - PACE_START) * spent // total
            pace[slot] = pace[slot] | value if slot in pace else value
        w_words = wqkv[p, 0]
        zero = zero_ref[0]
        for i in range(n_blocks):
            bands = []
            for c in range(n_ct):
                band = []
                for j in range(n_cols):
                    tile = w_words[c * LANES // 2:(c + 1) * LANES // 2, j * LANES:(j + 1) * LANES]
                    slot = (i * n_cols + j) * n_ct + c
                    if slot in pace:
                        top = tile[:SUBLANES, :] | (pace[slot] & zero)
                        tile = jnp.concatenate([top, tile[SUBLANES:, :]], axis=0)
                    band.append(tile)
                bands.append(jnp.concatenate(band, axis=1))
            lhs = x_words[pl.ds(i * PRE_ROWS // 2, PRE_ROWS // 2), :]
            qring[p, pl.ds(i * PRE_ROWS, PRE_ROWS), :] = _dot(
                pltpu.bitcast(lhs, BF16), pltpu.bitcast(jnp.concatenate(bands, axis=0), BF16))

        following = jnp.minimum(p + 1, n_pairs - 1)
        relayout(0, w_raw[w_slot(0, following)], following)
        ready = p >= kvo_lag
        late = jnp.where(ready, p - kvo_lag, p)
        for which in range(1, 4):
            relayout(which, w_raw[jnp.where(ready, w_slot(which, late), w_slot(0, p))], late)
        return carry

    def tile_prologue(c, carry):
        first = lambda c: (c * n_pairs) // n_ct
        forward_tile(c)
        return lax.fori_loop(first(c), first(c + 1), pair_prologue, carry)

    lax.fori_loop(0, n_ct, tile_prologue, 0)
    x_copy(1).wait()

    def inverse_tile(c, carry):
        late = n_pairs - kvo_lag + c
        wait(kvo_copies(late))
        spec = jnp.concatenate(
            [pltpu.bitcast(pspec[c, pl.ds(a * CHUNK, CHUNK), :], BF16) for a in range(n_chunks)],
            axis=1)
        y = _dot(inv_ref[...], spec)
        for a in range(n_chunks):
            t = pl.ds(a * CHUNK, CHUNK)
            pspec[c, t, :] = pltpu.bitcast(
                xs[t, _aligned(c * LANES, LANES)].astype(F32) * y[:, a * LANES:(a + 1) * LANES],
                I32)
        for which in range(1, 4):
            relayout(which, w_raw[w_slot(which, late)], late)
        return carry

    lax.fori_loop(0, n_ct, inverse_tile, 0)

    lane_lo = lax.broadcasted_iota(I32, (rows, LANES), 1) < (head_dim - LANES)
    col = lax.broadcasted_iota(I32, (rows, 2 * rows), 1)
    row = lax.broadcasted_iota(I32, (rows, 2 * rows), 0)
    head0 = col < rows
    key = jnp.where(head0, col, col - rows)
    visible = (row < n_mem) | (key >= seg) | (row - n_mem >= key)
    zeros = jnp.zeros((rows, LANES), F32)
    gate_w = gate_ref[...].astype(F32)
    gate_w = jnp.concatenate([gate_w[c:c + 1, :] for c in range(n_ct)], axis=1)

    def split_heads(a, b, c):
        top = jnp.concatenate([a, jnp.where(lane_lo, b, 0.0), zeros], axis=1)
        bottom = jnp.concatenate([zeros, jnp.where(lane_lo, 0.0, b), c], axis=1)
        return jnp.concatenate([top, bottom], axis=0).astype(BF16)

    def softmax_pair(s):
        s = jnp.where(visible, s * scale, -1000000000.0)
        m0 = jnp.max(jnp.where(head0, s, -jnp.inf), axis=1, keepdims=True)
        m1 = jnp.max(jnp.where(head0, -jnp.inf, s), axis=1, keepdims=True)
        e = jnp.exp(s - jnp.where(head0, m0, m1))
        l0 = jnp.sum(jnp.where(head0, e, 0.0), axis=1, keepdims=True)
        l1 = jnp.sum(jnp.where(head0, 0.0, e), axis=1, keepdims=True)
        return e / jnp.where(head0, l0, l1)

    def step(s, carry):
        mem, q_put, q_get = carry
        t = _aligned(s * seg, seg)
        xt = xs[t, :].astype(F32)
        h = jnp.concatenate([xt, mem], axis=0)
        hq = jnp.concatenate(
            [xs[_aligned(lead + s * q_new, q_new), :].astype(F32), mem], axis=0)

        def project(p, j):
            cols = pl.ds(j * LANES, LANES)
            w = lambda which: pltpu.bitcast(wqkv[p, which, :, cols], BF16)
            if p == 0 and j == 0:
                out = [0.0] * 3
                for c in range(n_ct):
                    ch = slice(c * LANES, (c + 1) * LANES)
                    out = [
                        out[which] + _dot(lhs[:, ch], w(which)[ch, :])
                        for which, lhs in enumerate((hq, h, h))]
            else:
                out = [_dot(lhs, w(which)) for which, lhs in enumerate((hq, h, h))]
            new = out[0]
            qring[p, _aligned(q_put, q_new), cols] = new[:q_new, :]
            q = jnp.concatenate([new[q_new:, :], qring[p, _aligned(q_get, seg), cols]], axis=0)
            return q, out[1], out[2]

        q, k, v, prob, o, parts = {}, {}, {}, {}, {}, []
        acc = None
        for op, i in _mxu_order(n_pairs):
            if op == "qkv":
                parts.append(project(i, len(parts)))
                if len(parts) == pw // LANES:
                    q[i] = jnp.concatenate([part[0] for part in parts], axis=1)
                    k[i] = split_heads(*[part[1] for part in parts])
                    v[i] = split_heads(*[part[2] for part in parts])
                    parts = []
            elif op == "s":
                prob[i] = softmax_pair(_dot(q.pop(i), k.pop(i), _NT))
            elif op == "pv":
                o[i] = _dot(prob.pop(i), v.pop(i))
            else:
                part = _dot(o.pop(i), pltpu.bitcast(wo[i], BF16))
                acc = part if acc is None else acc + part

        gate = jax.nn.sigmoid(jnp.sum(xt * gate_w, axis=1, keepdims=True))
        b = jnp.concatenate([pspec[c, t, :] for c in range(n_ct)], axis=1)
        res = gate * acc[n_mem:, :] + (1.0 - gate) * pltpu.bitcast(b, F32)
        obuf[t, :] = res.astype(BF16)
        pltpu.make_async_copy(obuf.at[t, :], out_hbm.at[t, :], out_sem).start()
        wrap = lambda pos: jnp.where(pos >= ring, pos - ring, pos)
        return acc[:n_mem, :].astype(BF16).astype(F32), wrap(q_put + q_new), wrap(q_get + seg)

    lax.fori_loop(
        0, n_seg, step, (mem0_ref[...].astype(F32), jnp.int32(lead), jnp.int32(0)),
        unroll=UNROLL)
    pltpu.make_async_copy(obuf, out_hbm, out_sem).wait()


@functools.partial(jax.jit, static_argnames=("A_seg_len",))
def pallas_gated_mix__memory_aug_recurrent_mem_tr__ssm_conv_h3__prompt_kernel(
    A_x: jax.Array,
    A_mem0: jax.Array,
    A_Wq: jax.Array,
    A_Wk: jax.Array,
    A_Wv: jax.Array,
    A_Wo: jax.Array,
    A_seg_len: int,
    B_q: jax.Array,
    B_k: jax.Array,
    B_v: jax.Array,
    B_shift_k: jax.Array,
    B_ssm_k: jax.Array,
    B_ssm_D: jax.Array,
    gate_w: jax.Array,
):
    del B_q
    batch, seq, dm = A_x.shape
    _, n_heads, head_dim = A_Wq.shape
    n_mem = A_mem0.shape[1]
    n_taps = B_shift_k.shape[1]
    seg = int(A_seg_len)
    n_ct = dm // LANES
    n_pairs = n_heads // 2
    pw = 2 * head_dim
    assert batch == 1 and 2 * head_dim == 3 * LANES and dm % LANES == 0
    assert n_pairs == CHUNK // SUBLANES and n_ct + 2 <= KVO_SLOTS
    assert seq % (UNROLL * seg) == 0 and seq % (2 * PRE_ROWS) == 0 and seg % 32 == 0
    assert n_mem % SUBLANES == 0 and 2 * (seg + n_mem) <= LANES and n_taps <= SUBLANES

    as_rows = lambda w: jnp.transpose(w, (1, 2, 0)).reshape(n_heads * head_dim, dm)
    fwd, inv = _dft_matrices()
    small = (
        A_mem0.reshape(n_mem, dm), B_shift_k.T, B_ssm_D.reshape(n_ct, LANES),
        gate_w.reshape(n_ct, LANES), fwd, inv)

    hbm = pl.BlockSpec(memory_space=pl.ANY)
    out = pl.pallas_call(
        functools.partial(_kernel, seg=seg, n_mem=n_mem, n_taps=n_taps, head_dim=head_dim),
        out_shape=jax.ShapeDtypeStruct((seq, dm), BF16),
        in_specs=[hbm] * (8 + len(small)),
        out_specs=hbm,
        scratch_shapes=[pltpu.VMEM(a.shape, BF16) for a in small] + [
            pltpu.VMEM((seq, dm), BF16),
            pltpu.VMEM((seq // 4, dm), I32),
            pltpu.VMEM((2, seq, LANES), BF16),
            pltpu.VMEM((2, seq, LANES), BF16),
            pltpu.VMEM((2, LANES, seq), BF16),
            pltpu.VMEM((Q_SLOTS + 3 * KVO_SLOTS, pw, dm), BF16),
            pltpu.VMEM((n_pairs, 3, dm // 2, pw), I32),
            pltpu.VMEM((n_pairs, pw // 2, dm), I32),
            pltpu.VMEM((SUBLANES, LANES), F32),
            pltpu.VMEM((2, 2 * seq, LANES), F32),
            pltpu.VMEM((2, 2 * seq, LANES), F32),
            pltpu.VMEM((n_ct, seq, LANES), I32),
            pltpu.VMEM((n_pairs, seq // 2 + seg, pw), F32),
            pltpu.VMEM((seq, dm), BF16),
            pltpu.SMEM((1,), I32),
            pltpu.SemaphoreType.DMA,
            pltpu.SemaphoreType.DMA((2,)),
            pltpu.SemaphoreType.DMA((2,)),
            pltpu.SemaphoreType.DMA((Q_SLOTS,)),
            pltpu.SemaphoreType.DMA((KVO_SLOTS,)),
            pltpu.SemaphoreType.DMA,
        ],
        compiler_params=pltpu.CompilerParams(
            vmem_limit_bytes=112 * 1024 * 1024, disable_bounds_checks=True),
        name="gated_mix_rmt_h3",
    )(
        A_x.reshape(seq, dm), B_k.reshape(seq, dm), B_v.reshape(seq, dm), B_ssm_k,
        as_rows(A_Wq), as_rows(A_Wk), as_rows(A_Wv), A_Wo.reshape(n_heads * head_dim, dm),
        *small,
    )
    return out.reshape(batch, seq, dm)
```
